```python
import os as _os
_os.environ.setdefault("JAX_PLATFORMS", "cpu")
import jax
import jax.numpy as jnp

def _softmax(x, axis=-1):
    return jax.nn.softmax(x, axis=axis)
def _gelu(x):
    return jax.nn.gelu(x, approximate=True)
def _silu(x):
    return jax.nn.silu(x)
def _sigmoid(x):
    return jax.nn.sigmoid(x)
def _layernorm(x, axis=-1, eps=1e-5):
    m = jnp.mean(x, axis=axis, keepdims=True)
    v = jnp.var(x, axis=axis, keepdims=True)
    return (x - m) / jnp.sqrt(v + eps)
def _scatter_add(tgt, idx, src, axis=0):
    return tgt.at[idx].add(src)
def _segment_sum(src, seg, n):
    return jax.ops.segment_sum(src, seg, n)
class _Rng:
    def __init__(self, key):
        self._k = key
    def _next(self):
        self._k, sub = jax.random.split(self._k)
        return sub
    def normal(self, shape):
        return jax.random.normal(self._next(), shape, dtype=jnp.bfloat16)
    def randint(self, lo, hi, shape):
        return jax.random.randint(self._next(), shape, lo, hi, dtype=jnp.int32)
    def uniform(self, shape, lo=0.0, hi=1.0):
        return jax.random.uniform(self._next(), shape, jnp.bfloat16, lo, hi)
    def permutation(self, n):
        return jax.random.permutation(self._next(), n)


kernel_name = 'concat_heads__gqa_block_cached__mha_block_cached__near_ridge'

def setup_inputs():
    _rng = _Rng(jax.random.key(int.from_bytes(__import__("os").urandom(4), "little")))
    _w = (lambda a: (lambda t: t.astype(jnp.bfloat16) if jnp.issubdtype(t.dtype, jnp.floating) else t)(jnp.asarray(a)))
    def _A_setup():
        B, Sq, D = 16, 32, 512
        Hq, Hkv, Sk, Dh = 32, 8, 512, 128
        assert Hq % Hkv == 0, (Hq, Hkv)
        return {
            "x": _w((lambda *s: _rng.normal(s) * 0.8)(B, Sq, D)),
            "k_cache": _w((lambda *s: _rng.normal(s) * 0.8)(B, Hkv, Sk, Dh)),
            "v_cache": _w((lambda *s: _rng.normal(s) * 0.05)(B, Hkv, Sk, Dh)),
            "wq": _w((lambda *s: _rng.normal(s) * 0.8)(D, Hq * Dh) * (D ** -0.5)),
            "wo": _w((lambda *s: _rng.normal(s) * 0.05)(Hq * Dh, D) * ((Hq * Dh) ** -0.5)),
        }
    _A_in = _A_setup()

    def _B_setup():
        B, Sq, D = 16, 32, 512
        H, Sk, Dh = 32, 512, 128
        return {
            "x": _w((lambda *s: _rng.normal(s) * 0.8)(B, Sq, D)),
            "k_cache": _w((lambda *s: _rng.normal(s) * 0.8)(B, H, Sk, Dh)),
            "v_cache": _w((lambda *s: _rng.normal(s) * 0.05)(B, H, Sk, Dh)),
            "wq": _w((lambda *s: _rng.normal(s) * 0.8)(D, H * Dh) * (D ** -0.5)),
            "wo": _w((lambda *s: _rng.normal(s) * 0.05)(H * Dh, D) * ((H * Dh) ** -0.5)),
        }
    _B_in = _B_setup()

    return {
        "A_x": _A_in["x"],
        "A_k_cache": _A_in["k_cache"],
        "A_v_cache": _A_in["v_cache"],
        "A_wq": _A_in["wq"],
        "A_wo": _A_in["wo"],
        "B_x": _B_in["x"],
        "B_k_cache": _B_in["k_cache"],
        "B_v_cache": _B_in["v_cache"],
        "B_wq": _B_in["wq"],
        "B_wo": _B_in["wo"],
    }

def reference(A_x, A_k_cache, A_v_cache, A_wq, A_wo, B_x, B_k_cache, B_v_cache, B_wq, B_wo):
    def _A_ref(x, k_cache, v_cache, wq, wo):
        B, Sq, D = x.shape
        Hq, Dh = 32, 128
        Hkv = k_cache.shape[1]
        rep = Hq // Hkv
        q = (lambda x, *d: x.transpose(*d))((x @ wq).reshape(B, Sq, Hq, Dh), 0, 2, 1, 3)
        k = jnp.repeat(k_cache, rep, axis=1)
        v = jnp.repeat(v_cache, rep, axis=1)
        scores = jnp.einsum("bhqd,bhkd->bhqk", q, k) * (Dh ** -0.5)
        p = _softmax(scores, axis=-1)
        o = jnp.einsum("bhqk,bhkd->bhqd", p, v)
        return (lambda x, *d: x.transpose(*d))(o, 0, 2, 1, 3).reshape(B, Sq, Hq * Dh) @ wo

    def _B_ref(x, k_cache, v_cache, wq, wo):
        B, Sq, D = x.shape
        H, Dh = 32, 128
        q = (lambda x, *d: x.transpose(*d))((x @ wq).reshape(B, Sq, H, Dh), 0, 2, 1, 3)
        scores = jnp.einsum("bhqd,bhkd->bhqk", q, k_cache) * (Dh ** -0.5)
        p = _softmax(scores, axis=-1)
        o = jnp.einsum("bhqk,bhkd->bhqd", p, v_cache)
        return (lambda x, *d: x.transpose(*d))(o, 0, 2, 1, 3).reshape(B, Sq, H * Dh) @ wo

    a = _A_ref(A_x, A_k_cache, A_v_cache, A_wq, A_wo)
    b = _B_ref(B_x, B_k_cache, B_v_cache, B_wq, B_wo)
    return jnp.concatenate([a, b], axis=-1)
```

```python
import functools
import math

import jax
import jax.numpy as jnp
import jax.experimental.pallas as pl
import jax.experimental.pallas.tpu as pltpu

NT = (((1,), (1,)), ((), ()))
NN = (((1,), (0,)), ((), ()))

B, SQ, D = 16, 32, 512
H, HKV, SK, DH = 32, 8, 512, 128
REP = H // HKV
G = 4
M = G * SQ
NG = B // G
NSUP = NG * HKV
NS = 1 + REP
CH = 128
QSCALE = float(DH ** -0.5 * math.log2(math.e))


def build(L=3, order="jb_kv", do_compute=True, do_dma=True, name="fused_attn", ch=CH):

    def kernel(xa_h, ka_h, va_h, wqa_h, woa_h, xb_h, kb_h, vb_h, wqb_h, wob_h, out_h,
               xa, xb, wqa, wqb, woa, wob, qa, qb, oa, ob, acca, accb, obuf,
               k0, k1, k2, k3, k4, v0, v1, v2, v3, v4, ksem, vsem, wsem, osem):
        kbuf = (k0, k1, k2, k3, k4)
        vbuf = (v0, v1, v2, v3, v4)

        class Prio:
            n = 0

        def start(src, dst, sem):
            pltpu.make_async_copy(src, dst, sem).start(priority=Prio.n % 2)
            Prio.n += 1

        def issue(n, s):
            if not do_dma:
                return
            g = n // HKV
            j = n % HKV
            if s == 0:
                ksrc, vsrc, h = ka_h, va_h, j
            else:
                ksrc, vsrc, h = kb_h, vb_h, j * REP + (s - 1)
            nj = SK // ch
            items = []
            if order == "jb_kv":
                for c in range(nj):
                    for b in range(G):
                        items += [(0, b, c), (1, b, c)]
            elif order == "kv_jb":
                for kv in range(2):
                    for c in range(nj):
                        for b in range(G):
                            items.append((kv, b, c))
            elif order == "bj_kv":
                for b in range(G):
                    for c in range(nj):
                        items += [(0, b, c), (1, b, c)]
            for kv, b, c in items:
                src = (ksrc, vsrc)[kv].at[g * G + b, h, pl.ds(c * ch, ch)]
                dst = (kbuf, vbuf)[kv][s].at[b, pl.ds(c * ch, ch)]
                start(src, dst, (ksem, vsem)[kv].at[s])

        def wait_k(s):
            if do_dma:
                pltpu.make_async_copy(kbuf[s], kbuf[s], ksem.at[s]).wait()

        def wait_v(s):
            if do_dma:
                pltpu.make_async_copy(vbuf[s], vbuf[s], vsem.at[s]).wait()

        def w_body(i, _):
            for c in range(4):
                r = pl.multiple_of(i * 16 + (c // 2) * 8, 8)
                cols = pl.ds((c % 2) * 2048, 2048)
                start(wqa_h.at[pl.ds(r, 8), cols], wqa.at[pl.ds(r, 8), cols], wsem.at[0])
                start(wqb_h.at[pl.ds(r, 8), cols], wqb.at[pl.ds(r, 8), cols], wsem.at[1])
                r2 = pl.ds(pl.multiple_of(i * 128 + c * 32, 32), 32)
                start(woa_h.at[r2], woa.at[r2], wsem.at[2])
                start(wob_h.at[r2], wob.at[r2], wsem.at[3])

        for b in range(B):
            start(xa_h.at[b], xa.at[b], wsem.at[4])
            start(xb_h.at[b], xb.at[b], wsem.at[5])
        jax.lax.fori_loop(0, 32, w_body, None)
        for s in range(L):
            issue(0, s)
        for i, r in enumerate((wqa, wqb, woa, wob, xa, xb)):
            pltpu.make_async_copy(r, r, wsem.at[i]).wait()

        def qproj(n, i):
            g = n // HKV
            j = n % HKV
            col = pl.ds(pl.multiple_of((j * REP + i) * DH, DH), DH)
            for x, w, q in ((xa, wqa, qa), (xb, wqb, qb)):
                xg = x[pl.ds(g * G, G)].reshape(M, D)
                r = jax.lax.dot_general(xg, w[:, col], NN, preferred_element_type=jnp.float32)
                q[i] = (r * QSCALE).astype(jnp.bfloat16)

        def oproj(n, i, o, w, acc):
            j = n % HKV
            row = pl.ds(pl.multiple_of((j * REP + i) * DH, DH), DH)
            acc[...] += jax.lax.dot_general(o[i], w[row, :], NN, preferred_element_type=jnp.float32)

        def scores(q, k):
            s = jax.lax.dot_general(q, k, NT, preferred_element_type=jnp.float32)
            m = jnp.max(s, axis=-1, keepdims=True)
            p = jnp.exp2(s - m)
            l = jnp.sum(p, axis=-1, keepdims=True)
            return p.astype(jnp.bfloat16), 1.0 / l

        def pv(p, r, v):
            o = jax.lax.dot_general(p, v, NN, preferred_element_type=jnp.float32)
            return (o * r).astype(jnp.bfloat16)

        acca[...] = jnp.zeros_like(acca)
        accb[...] = jnp.zeros_like(accb)
        if do_compute:
            for i in range(REP):
                qproj(0, i)

        def body(n, _):
            nn = jnp.minimum(n + 1, NSUP - 1)
            for s in range(NS):
                wait_k(s)
                t = s + L
                if t < NS:
                    issue(n, t)
                else:
                    @pl.when(n + 1 < NSUP)
                    def _():
                        issue(n + 1, t - NS)
                if not do_compute:
                    wait_v(s)
                    continue
                if s == 0:
                    ps = []
                    for b in range(G):
                        q = jnp.concatenate([qa[i, pl.ds(b * SQ, SQ), :] for i in range(REP)], axis=0)
                        ps.append(scores(q, kbuf[s][b]))
                    wait_v(s)
                    for b in range(G):
                        o = pv(*ps[b], vbuf[s][b])
                        for i in range(REP):
                            oa[i, pl.ds(b * SQ, SQ), :] = o[i * SQ:(i + 1) * SQ]
                else:
                    i = s - 1
                    ps = [scores(qb[i, pl.ds(b * SQ, SQ), :], kbuf[s][b]) for b in range(G)]
                    qproj(nn, i)
                    oproj(n, i, oa, woa, acca)
                    if i > 0:
                        oproj(n, i - 1, ob, wob, accb)
                    wait_v(s)
                    for b in range(G):
                        ob[i, pl.ds(b * SQ, SQ), :] = pv(*ps[b], vbuf[s][b])
                    if i == REP - 1:
                        oproj(n, i, ob, wob, accb)

            @pl.when(n % HKV == HKV - 1)
            def _():
                g = n // HKV
                rows = pl.ds(g * G, G)
                obuf[rows, :, 0:D] = acca[...].astype(jnp.bfloat16).reshape(G, SQ, D)
                obuf[rows, :, D:2 * D] = accb[...].astype(jnp.bfloat16).reshape(G, SQ, D)
                acca[...] = jnp.zeros_like(acca)
                accb[...] = jnp.zeros_like(accb)
                for b in range(G):
                    for c in range(2):
                        rr = pl.ds(c * 16, 16)
                        start(obuf.at[g * G + b, rr], out_h.at[g * G + b, rr], osem)

        jax.lax.fori_loop(0, NSUP, body, None)
        pltpu.make_async_copy(obuf, out_h, osem).wait()

    bf = jnp.bfloat16
    scratch = [
        pltpu.VMEM((B, SQ, D), bf), pltpu.VMEM((B, SQ, D), bf),
        pltpu.VMEM((D, H * DH), bf), pltpu.VMEM((D, H * DH), bf),
        pltpu.VMEM((H * DH, D), bf), pltpu.VMEM((H * DH, D), bf),
        pltpu.VMEM((REP, M, DH), bf), pltpu.VMEM((REP, M, DH), bf),
        pltpu.VMEM((REP, M, DH), bf), pltpu.VMEM((REP, M, DH), bf),
        pltpu.VMEM((M, D), jnp.float32), pltpu.VMEM((M, D), jnp.float32),
        pltpu.VMEM((B, SQ, 2 * D), bf),
    ] + [pltpu.VMEM((G, SK, DH), bf)] * (2 * NS) + [
        pltpu.SemaphoreType.DMA((NS,)), pltpu.SemaphoreType.DMA((NS,)),
        pltpu.SemaphoreType.DMA((6,)), pltpu.SemaphoreType.DMA,
    ]

    @jax.jit
    def f(A_x, A_k_cache, A_v_cache, A_wq, A_wo, B_x, B_k_cache, B_v_cache, B_wq, B_wo):
        return pl.pallas_call(
            kernel,
            in_specs=[pl.BlockSpec(memory_space=pl.ANY)] * 10,
            out_specs=pl.BlockSpec(memory_space=pl.ANY),
            out_shape=jax.ShapeDtypeStruct((B, SQ, 2 * D), bf),
            scratch_shapes=scratch,
            compiler_params=pltpu.CompilerParams(vmem_limit_bytes=100 * 1024 * 1024),
            name=name,
        )(A_x, A_k_cache, A_v_cache, A_wq, A_wo, B_x, B_k_cache, B_v_cache, B_wq, B_wo)

    return f


_impl = build()


@jax.jit
def pallas_concat_heads__gqa_block_cached__mha_block_cached__near_ridge_kernel(
    A_x, A_k_cache, A_v_cache, A_wq, A_wo, B_x, B_k_cache, B_v_cache, B_wq, B_wo
):
    return _impl(A_x, A_k_cache, A_v_cache, A_wq, A_wo, B_x, B_k_cache, B_v_cache, B_wq, B_wo)
```

```python
import math

import jax
import jax.numpy as jnp
import jax.experimental.pallas as pl
import jax.experimental.pallas.tpu as pltpu

_NT = (((1,), (1,)), ((), ()))
_NN = (((1,), (0,)), ((), ()))

B, SQ, D = 16, 32, 512
H, HKV, SK, DH = 32, 8, 512, 128
REP = H // HKV
G = 4
M = G * SQ
NG = B // G
ROUNDS = NG * HKV
STEPS = 1 + REP
AHEAD = STEPS - 1
KV_ROWS = 128
ISSUE_ORDER = (0, 1, 3, 2)
SCORE_SCALE = DH ** -0.5 * math.log2(math.e)

PROJECTIONS = (
    (("qb", 0),),
    (("qb", 1), ("qa", 0), ("oa", 0), ("oa", 1)),
    (("qb", 2), ("qa", 1), ("qa", 2), ("oa", 2), ("ob", 0)),
    (("qb", 3), ("qa", 3), ("oa", 3), ("ob", 1)),
    (("ob", 2),),
)


def _batch(g, i):
    return (g % 2) + 8 * (g // 2) + 2 * i


def _start(src, dst, sem, priority):
    pltpu.make_async_copy(src, dst, sem).start(priority=priority)


def _wait_filled(buf, sem):
    pltpu.make_async_copy(buf, buf, sem).wait()


def _softmax_numerator(q, k):
    s = jax.lax.dot_general(q, k, _NT, preferred_element_type=jnp.float32)
    p = jnp.exp2((s - jnp.max(s, axis=-1, keepdims=True)) * SCORE_SCALE)
    return p.astype(jnp.bfloat16), 1.0 / jnp.sum(p, axis=-1, keepdims=True)


def _weighted_values(p, inv_sum, v):
    o = jax.lax.dot_general(p, v, _NN, preferred_element_type=jnp.float32)
    return (o * inv_sum).astype(jnp.bfloat16)


def _stream(xa_hbm, ka_hbm, va_hbm, wqa_hbm, woa_hbm,
            xb_hbm, kb_hbm, vb_hbm, wqb_hbm, wob_hbm, out_hbm,
            xa, xb, wqa, wqb, woa, wob, qa, qb, oa, ob, acc_a, acc_b, out_buf,
            k_slots, v_slots, out_sem, k_sems, v_sems, w_sems):
    def fetch_kv(n, s):
        g, j = n // HKV, n % HKV
        if s == 0:
            k_hbm, v_hbm, head = ka_hbm, va_hbm, j
        else:
            k_hbm, v_hbm, head = kb_hbm, vb_hbm, j * REP + (s - 1)
        for c in range(SK // KV_ROWS):
            rows = pl.ds(c * KV_ROWS, KV_ROWS)
            for i in ISSUE_ORDER:
                b = _batch(g, i)
                _start(k_hbm.at[b, head, rows], k_slots[s].at[i, rows], k_sems.at[s], 0)
                _start(v_hbm.at[b, head, rows], v_slots[s].at[i, rows], v_sems.at[s], 1)

    def fetch_wq(src, dst, sem, blk, priority):
        rows = pl.ds(pl.multiple_of((blk // 2) * 8, 8), 8)
        cols = pl.ds(pl.multiple_of((blk % 2) * 2048, 2048), 2048)
        _start(src.at[rows, cols], dst.at[rows, cols], sem, priority)

    def fetch_wo(src, dst, sem, blk, priority):
        rows = pl.ds(pl.multiple_of(blk * 32, 32), 32)
        _start(src.at[rows], dst.at[rows], sem, priority)

    def fetch_weights(i, carry):
        for u in range(4):
            for half in range(2):
                blk = half * 64 + i * 4 + u
                fetch_wq(wqa_hbm, wqa, w_sems.at[0], blk, 0)
                fetch_wq(wqb_hbm, wqb, w_sems.at[1], blk, 1)
                fetch_wo(woa_hbm, woa, w_sems.at[2], blk, 0)
                fetch_wo(wob_hbm, wob, w_sems.at[3], blk, 1)
        b = _batch(i // G, i % G)
        _start(xa_hbm.at[b], xa.at[i], w_sems.at[4], 0)
        _start(xb_hbm.at[b], xb.at[i], w_sems.at[5], 1)
        return carry

    def head_slice(n, i):
        return pl.ds(pl.multiple_of(((n % HKV) * REP + i) * DH, DH), DH)

    def project_q(n, i, x, wq, q):
        xg = x[pl.ds((n // HKV) * G, G)].reshape(M, D)
        r = jax.lax.dot_general(xg, wq[:, head_slice(n, i)], _NN,
                                preferred_element_type=jnp.float32)
        q[i] = r.astype(jnp.bfloat16)

    def project_o(n, i, o, wo, acc, half):
        r = jax.lax.dot_general(o[i], wo[head_slice(n, i), :], _NN,
                                preferred_element_type=jnp.float32)
        prev = acc[...]
        if i == 0:
            prev = jnp.where(n % HKV == 0, 0.0, prev)
        r = prev + r
        acc[...] = r
        if i == REP - 1:
            out_buf[pl.ds((n // HKV) * G, G), :, half * D:(half + 1) * D] = (
                r.astype(jnp.bfloat16).reshape(G, SQ, D))

    def write_group(g):
        for i in range(G):
            for c in range(2):
                rows = pl.ds(c * (SQ // 2), SQ // 2)
                _start(out_buf.at[g * G + i, rows], out_hbm.at[_batch(g, i), rows], out_sem, c)

    jax.lax.fori_loop(0, B, fetch_weights, None)
    for s in range(AHEAD):
        fetch_kv(0, s)
    for i, buf in enumerate((wqa, wqb, woa, wob, xa, xb)):
        _wait_filled(buf, w_sems.at[i])

    acc_a[...] = jnp.zeros_like(acc_a)
    acc_b[...] = jnp.zeros_like(acc_b)
    for i in range(REP):
        project_q(0, i, xa, wqa, qa)

    def one_round(n, carry):
        nxt = jnp.minimum(n + 1, ROUNDS - 1)
        for s in range(STEPS):
            _wait_filled(k_slots[s], k_sems.at[s])
            if s + AHEAD < STEPS:
                fetch_kv(n, s + AHEAD)
            else:
                @pl.when(n + 1 < ROUNDS)
                def _():
                    fetch_kv(n + 1, s + AHEAD - STEPS)
            if s == STEPS - 1:
                @pl.when(n == ROUNDS - 1)
                def _():
                    for g in range(NG - 1):
                        write_group(g)

            probs = []
            for i in range(G):
                rows = pl.ds(i * SQ, SQ)
                if s == 0:
                    q = jnp.concatenate([qa[h, rows, :] for h in range(REP)], axis=0)
                else:
                    q = qb[s - 1, rows, :]
                probs.append(_softmax_numerator(q, k_slots[s][i]))

            for kind, h in PROJECTIONS[s]:
                if kind == "qa":
                    project_q(nxt, h, xa, wqa, qa)
                elif kind == "qb":
                    project_q(n, h, xb, wqb, qb)
                elif kind == "oa":
                    project_o(n, h, oa, woa, acc_a, 0)
                else:
                    project_o(n, h, ob, wob, acc_b, 1)

            _wait_filled(v_slots[s], v_sems.at[s])
            for i in range(G):
                rows = pl.ds(i * SQ, SQ)
                o = _weighted_values(*probs[i], v_slots[s][i])
                if s == 0:
                    for h in range(REP):
                        oa[h, rows, :] = o[h * SQ:(h + 1) * SQ]
                else:
                    ob[s - 1, rows, :] = o
            if s == STEPS - 1:
                project_o(n, REP - 1, ob, wob, acc_b, 1)
        return carry

    jax.lax.fori_loop(0, ROUNDS, one_round, None)
    write_group(NG - 1)


def _kernel(*refs):
    fixed, slots, out_sem = refs[:24], refs[24:-1], refs[-1]
    out_hbm, out_buf = fixed[10], fixed[23]
    pl.run_scoped(
        lambda k_sems, v_sems, w_sems: _stream(
            *fixed, slots[:STEPS], slots[STEPS:], out_sem, k_sems, v_sems, w_sems),
        pltpu.SemaphoreType.DMA((STEPS,)),
        pltpu.SemaphoreType.DMA((STEPS,)),
        pltpu.SemaphoreType.DMA((6,)),
    )
    pltpu.make_async_copy(out_buf, out_hbm, out_sem).wait()


@jax.jit
def pallas_concat_heads__gqa_block_cached__mha_block_cached__near_ridge_kernel(
    A_x: jax.Array,
    A_k_cache: jax.Array,
    A_v_cache: jax.Array,
    A_wq: jax.Array,
    A_wo: jax.Array,
    B_x: jax.Array,
    B_k_cache: jax.Array,
    B_v_cache: jax.Array,
    B_wq: jax.Array,
    B_wo: jax.Array,
):
    assert A_x.shape == B_x.shape == (B, SQ, D)
    assert A_k_cache.shape == A_v_cache.shape == (B, HKV, SK, DH)
    assert B_k_cache.shape == B_v_cache.shape == (B, H, SK, DH)
    assert A_wq.shape == B_wq.shape == (D, H * DH)
    assert A_wo.shape == B_wo.shape == (H * DH, D)

    bf16 = jnp.bfloat16
    scratch_shapes = (
        [pltpu.VMEM((B, SQ, D), bf16)] * 2
        + [pltpu.VMEM((D, H * DH), bf16)] * 2
        + [pltpu.VMEM((H * DH, D), bf16)] * 2
        + [pltpu.VMEM((REP, M, DH), bf16)] * 4
        + [pltpu.VMEM((M, D), jnp.float32)] * 2
        + [pltpu.VMEM((B, SQ, 2 * D), bf16)]
        + [pltpu.VMEM((G, SK, DH), bf16)] * (2 * STEPS)
        + [pltpu.SemaphoreType.DMA]
    )
    return pl.pallas_call(
        _kernel,
        in_specs=[pl.BlockSpec(memory_space=pl.ANY)] * 10,
        out_specs=pl.BlockSpec(memory_space=pl.ANY),
        out_shape=jax.ShapeDtypeStruct((B, SQ, 2 * D), bf16),
        scratch_shapes=scratch_shapes,
        compiler_params=pltpu.CompilerParams(vmem_limit_bytes=64 * 1024 * 1024),
        name="fused_gqa_mha",
    )(A_x, A_k_cache, A_v_cache, A_wq, A_wo, B_x, B_k_cache, B_v_cache, B_wq, B_wo)
```
